```python
import os as _os
_os.environ.setdefault("JAX_PLATFORMS", "cpu")
import jax
import jax.numpy as jnp

def _softmax(x, axis=-1):
    return jax.nn.softmax(x, axis=axis)
def _gelu(x):
    return jax.nn.gelu(x, approximate=True)
def _silu(x):
    return jax.nn.silu(x)
def _sigmoid(x):
    return jax.nn.sigmoid(x)
def _layernorm(x, axis=-1, eps=1e-5):
    m = jnp.mean(x, axis=axis, keepdims=True)
    v = jnp.var(x, axis=axis, keepdims=True)
    return (x - m) / jnp.sqrt(v + eps)
def _scatter_add(tgt, idx, src, axis=0):
    return tgt.at[idx].add(src)
def _segment_sum(src, seg, n):
    return jax.ops.segment_sum(src, seg, n)
class _Rng:
    def __init__(self, key):
        self._k = key
    def _next(self):
        self._k, sub = jax.random.split(self._k)
        return sub
    def normal(self, shape):
        return jax.random.normal(self._next(), shape, dtype=jnp.bfloat16)
    def randint(self, lo, hi, shape):
        return jax.random.randint(self._next(), shape, lo, hi, dtype=jnp.int32)
    def uniform(self, shape, lo=0.0, hi=1.0):
        return jax.random.uniform(self._next(), shape, jnp.bfloat16, lo, hi)
    def permutation(self, n):
        return jax.random.permutation(self._next(), n)


kernel_name = 'standalone__groupnorm__sampling'

def setup_inputs():
    _rng = _Rng(jax.random.key(int.from_bytes(__import__("os").urandom(4), "little")))
    _w = (lambda a: (lambda t: t.astype(jnp.bfloat16) if jnp.issubdtype(t.dtype, jnp.floating) else t)(jnp.asarray(a)))
    B = 32
    G = 32
    cpg = max(1, 576 // G)
    C = G * cpg
    H, W = 32, 16
    return {
        "x": _w((lambda *s: _rng.normal(s) * 0.05)(B, C, H, W)),
        "g": _w((lambda *s: _rng.normal(s) * 0.05)(C) + 1.0),
        "b": _w((lambda *s: _rng.normal(s) * 0.05)(C)),
    }

def reference(x, g, b):
    G = 32
    B, C, H, W = x.shape[0], x.shape[1], x.shape[2], x.shape[3]
    xr = x.reshape(B, G, C // G, H, W)
    mu = xr.mean(axis=(2, 3, 4), keepdims=True)
    var = ((xr - mu) ** 2).mean(axis=(2, 3, 4), keepdims=True)
    xn = (xr - mu) / jnp.sqrt(var + 1e-5)
    xn = xn.reshape(B, C, H, W)
    return xn * g[None, :, None, None] + b[None, :, None, None]
```

```python
import jax
import jax.numpy as jnp
from jax import lax
import jax.experimental.pallas as pl
import jax.experimental.pallas.tpu as pltpu

_GROUPS = 32
_EPS = 1e-5
_ROWS = 8
_WRITE_ROWS = 40
_LATE_SAMPLES = 8
_TAIL_ROWS = 256


@jax.jit
def pallas_standalone__groupnorm__sampling_kernel(
    x: jax.Array,
    g: jax.Array,
    b: jax.Array,
):
    B, C, H, W = x.shape
    HW = H * W
    cpg = C // _GROUPS
    last = B - 1
    split = B - _LATE_SAMPLES
    head = HW - _TAIL_ROWS

    def kernel(x_hbm, g_hbm, b_hbm, o_hbm, xbuf, obuf, gbuf, bbuf, rsem, tsem, psem, wsem):
        def read(i):
            return pltpu.make_async_copy(x_hbm.at[i], xbuf.at[i], rsem.at[i])

        read_head = pltpu.make_async_copy(
            x_hbm.at[last, pl.ds(0, head)], xbuf.at[last, pl.ds(0, head)], tsem.at[0])
        read_tail = pltpu.make_async_copy(
            x_hbm.at[last, pl.ds(head, _TAIL_ROWS)], xbuf.at[last, pl.ds(head, _TAIL_ROWS)], tsem.at[1])
        read_g = pltpu.make_async_copy(g_hbm, gbuf, psem.at[0])
        read_b = pltpu.make_async_copy(b_hbm, bbuf, psem.at[1])

        read(0).start()
        read_g.start()
        read_b.start()

        @pl.loop(1, last)
        def _(i):
            read(i).start()

        read_head.start()
        read_tail.start()
        read_g.wait()
        read_b.wait()

        gamma = gbuf[...].astype(jnp.float32).reshape(1, C)
        beta = bbuf[...].astype(jnp.float32).reshape(1, C)
        first = lax.broadcasted_iota(jnp.int32, (_GROUPS, C), 0) * cpg
        chan = lax.broadcasted_iota(jnp.int32, (_GROUPS, C), 1)
        member = (chan >= first) & (chan < first + cpg)
        inv_n = 1.0 / (HW * cpg)

        def group_mean(acc):
            cols = jnp.sum(acc, axis=0, keepdims=True)
            return jnp.sum(jnp.where(member, cols, 0.0), axis=1, keepdims=True) * inv_n

        def per_channel(v):
            return jnp.sum(jnp.where(member, v, 0.0), axis=0, keepdims=True)

        def normalise(i):
            def rows(j):
                return pl.ds(pl.multiple_of(j * _ROWS, _ROWS), _ROWS)

            def load(j):
                return xbuf[i, rows(j), :].astype(jnp.float32)

            steps = HW // _ROWS
            zero = jnp.zeros((_ROWS, C), jnp.float32)
            total = lax.fori_loop(0, steps, lambda j, a: a + load(j), zero, unroll=8)
            mean = jnp.broadcast_to(per_channel(group_mean(total)), (_ROWS, C))

            def add_square(j, a):
                d = load(j) - mean
                return a + d * d

            squares = lax.fori_loop(0, steps, add_square, zero, unroll=8)
            rstd = per_channel(lax.rsqrt(group_mean(squares) + _EPS))
            scale = jnp.broadcast_to(rstd * gamma, (_ROWS, C))
            shift = jnp.broadcast_to(beta, (_ROWS, C))

            @pl.loop(0, steps, unroll=8)
            def _(j):
                obuf[i, rows(j), :] = ((load(j) - mean) * scale + shift).astype(obuf.dtype)

        def write(lo, hi):
            for r in range(0, HW, _WRITE_ROWS):
                idx = (pl.ds(lo, hi - lo), pl.ds(r, min(_WRITE_ROWS, HW - r)))
                pltpu.make_async_copy(obuf.at[idx], o_hbm.at[idx], wsem).start()

        @pl.loop(0, split)
        def _(i):
            read(i).wait()
            normalise(i)

        read_head.wait()
        write(0, split)

        @pl.loop(split, B)
        def _(i):
            @pl.when(i < last)
            def _():
                read(i).wait()

            @pl.when(i == last)
            def _():
                read_tail.wait()

            normalise(i)

        write(split, B)
        pltpu.make_async_copy(obuf, o_hbm, wsem).wait()

    xt = x.transpose(0, 2, 3, 1).reshape(B, HW, C)
    out = pl.pallas_call(
        kernel,
        in_specs=[pl.BlockSpec(memory_space=pltpu.HBM)] * 3,
        out_specs=pl.BlockSpec(memory_space=pltpu.HBM),
        out_shape=jax.ShapeDtypeStruct((B, HW, C), x.dtype),
        scratch_shapes=[
            pltpu.VMEM((B, HW, C), x.dtype),
            pltpu.VMEM((B, HW, C), x.dtype),
            pltpu.VMEM((C,), g.dtype),
            pltpu.VMEM((C,), b.dtype),
            pltpu.SemaphoreType.DMA((last,)),
            pltpu.SemaphoreType.DMA((2,)),
            pltpu.SemaphoreType.DMA((2,)),
            pltpu.SemaphoreType.DMA(()),
        ],
        compiler_params=pltpu.CompilerParams(
            vmem_limit_bytes=64 * 2**20, disable_semaphore_checks=True),
    )(xt, g, b)
    return out.reshape(B, H, W, C).transpose(0, 3, 1, 2)
```

```python
import jax
import jax.numpy as jnp
from jax import lax
import jax.experimental.pallas as pl
import jax.experimental.pallas.tpu as pltpu

_GROUPS = 32
_EPS = 1e-5

_SETS = 4
_ROWS = 8
_READ_ROWS = 24
_WRITE_ROWS = 24
_TAIL_ROWS = 40
_EARLY_SETS = 2
_WIDE = 6
_SIDE_ROWS = 112
_SIDE_SKIP = 32
_SIDE_REUSE = 48


@jax.jit
def pallas_standalone__groupnorm__sampling_kernel(
    x: jax.Array,
    g: jax.Array,
    b: jax.Array,
):
    B, C, H, W = x.shape
    HW = H * W
    cpg = C // _GROUPS
    P = B // _SETS
    last = _SETS - 1
    side_start = HW - _SIDE_ROWS
    tail_start = side_start - _TAIL_ROWS
    shape = (P, _SETS, HW, C)

    order = [(j + _WIDE) % P for j in range(P)]

    side_first = (0, side_start, _SIDE_REUSE, 0)
    side_middle = [(0, side_start + _SIDE_REUSE, _SIDE_ROWS - _SIDE_REUSE, _SIDE_REUSE)]
    side_middle += [(j, side_start, _SIDE_ROWS, j * _SIDE_ROWS) for j in range(1, P - 1)]
    side_middle += [(P - 1, side_start + _SIDE_SKIP,
                     _SIDE_ROWS - _SIDE_SKIP - _SIDE_REUSE, (P - 1) * _SIDE_ROWS)]
    side_again = (P - 1, HW - _SIDE_REUSE, _SIDE_REUSE, 0)
    side_late = side_middle + [side_again]
    smem_rows = P * _SIDE_ROWS - _SIDE_SKIP - _SIDE_REUSE

    def kernel(x_hbm, g_hbm, b_hbm, o_hbm, xbuf, obuf, gbuf, bbuf, side,
               set_sem, tail_sem, skip_sem, param_sem, fill_sem, drain_sem, out_sem):
        def read(k, row, n, sem):
            idx = (slice(None), k, pl.ds(row, n))
            return pltpu.make_async_copy(x_hbm.at[idx], xbuf.at[idx], sem)

        def fill(piece, sem):
            j, row, n, slot = piece
            return pltpu.make_async_copy(
                x_hbm.at[order[j], last, pl.ds(row, n)], side.at[pl.ds(slot, n)], sem)

        def drain(piece, sem):
            j, row, n, slot = piece
            return pltpu.make_async_copy(
                side.at[pl.ds(slot, n)], xbuf.at[order[j], last, pl.ds(row, n)], sem)

        def start_rows(copy, lo, hi, step):
            whole = (hi - lo) // step

            @pl.loop(0, whole)
            def _(j):
                copy(pl.multiple_of(lo + j * step, _ROWS), step).start()

            rest = lo + whole * step
            if rest < hi:
                copy(rest, hi - rest).start()

        def start_in_order(copies):
            @pl.loop(0, len(copies))
            def _(j):
                for n, copy in enumerate(copies):
                    pl.when(j == n)(lambda copy=copy: copy().start())

        def start_set(k, lo, hi):
            start_rows(lambda row, n: read(k, row, n, set_sem.at[k]), lo, hi, _READ_ROWS)

        def start_write(samples, sets):
            def write(row, n):
                idx = (samples, sets, pl.ds(row, n))
                return pltpu.make_async_copy(obuf.at[idx], o_hbm.at[idx], out_sem)

            start_rows(write, 0, HW, _WRITE_ROWS)

        read_g = pltpu.make_async_copy(g_hbm, gbuf, param_sem.at[0])
        read_b = pltpu.make_async_copy(b_hbm, bbuf, param_sem.at[1])
        skipped = (order[-1], last, pl.ds(side_start, _SIDE_SKIP))
        read_skipped = pltpu.make_async_copy(x_hbm.at[skipped], xbuf.at[skipped], skip_sem)

        read(0, 0, _READ_ROWS, set_sem.at[0]).start()
        read_g.start()
        read_b.start()
        start_in_order([lambda: fill(side_first, fill_sem.at[0])]
                       + [lambda p=p: fill(p, fill_sem.at[1]) for p in side_middle])
        start_set(0, _READ_ROWS, HW)
        start_set(1, 0, HW)
        fill(side_first, fill_sem.at[0]).wait()
        drain(side_first, fill_sem.at[0]).start()
        drain(side_first, fill_sem.at[0]).wait()
        fill(side_again, fill_sem.at[1]).start()
        read_skipped.start()
        for k in range(2, last):
            start_set(k, 0, HW)
        start_set(last, 0, tail_start)
        start_rows(lambda row, n: read(last, row, n, tail_sem), tail_start, side_start, _READ_ROWS)

        read_g.wait()
        read_b.wait()
        gamma = gbuf[...].astype(jnp.float32).reshape(1, C)
        beta = bbuf[...].astype(jnp.float32).reshape(1, C)
        first = lax.broadcasted_iota(jnp.int32, (_GROUPS, C), 0) * cpg
        chan = lax.broadcasted_iota(jnp.int32, (_GROUPS, C), 1)
        member = (chan >= first) & (chan < first + cpg)

        def group_mean(partial):
            cols = jnp.sum(partial, axis=0, keepdims=True)
            return jnp.sum(jnp.where(member, cols, 0.0), axis=1, keepdims=True) / (HW * cpg)

        def per_channel(v):
            return jnp.sum(jnp.where(member, v, 0.0), axis=0, keepdims=True)

        def normalise(src, dst):
            steps = [pl.ds(row, _ROWS) for row in range(0, HW, _ROWS)]

            total = jnp.zeros((_ROWS, C), jnp.float32)
            for rows in steps:
                total += src[rows, :].astype(jnp.float32)
            mean = jnp.broadcast_to(per_channel(group_mean(total)), (_ROWS, C))

            squares = jnp.zeros((_ROWS, C), jnp.float32)
            for rows in steps:
                d = src[rows, :].astype(jnp.float32) - mean
                squares += d * d
            rstd = per_channel(lax.rsqrt(group_mean(squares) + _EPS))

            scale = jnp.broadcast_to(rstd * gamma, (_ROWS, C))
            shift = jnp.broadcast_to(beta, (_ROWS, C))
            for rows in steps:
                d = src[rows, :].astype(jnp.float32) - mean
                dst[rows, :] = (d * scale + shift).astype(dst.dtype)

        wide = pl.ds(0, _WIDE)

        @pl.loop(0, B)
        def _(t):
            k = t // P
            j = t % P

            @pl.when((j == 0) & (k < last))
            def _():
                read(k, 0, HW, set_sem.at[k]).wait()

            @pl.when(t == _EARLY_SETS * P)
            def _():
                for p in side_late:
                    fill(p, fill_sem.at[1]).wait()
                start_in_order([lambda p=p: drain(p, drain_sem.at[p[0]]) for p in side_late])
                read_skipped.wait()
                read(last, 0, tail_start, set_sem.at[last]).wait()
                for early in range(_EARLY_SETS):
                    start_write(wide, pl.ds(early, 1))
                read(last, tail_start, _TAIL_ROWS, tail_sem).wait()

            for step in range(P):
                @pl.when(t == last * P + step)
                def _():
                    for p in side_late:
                        if p[0] == step:
                            drain(p, drain_sem.at[step]).wait()

            i = (t + _WIDE) % P
            normalise(xbuf.at[i, k], obuf.at[i, k])

            @pl.when((j == P - 1) & (k >= _EARLY_SETS))
            def _():
                start_write(wide, pl.ds(k, 1))

            @pl.when(t == last * P + (P - _WIDE) - 1)
            def _():
                start_write(pl.ds(_WIDE, P - _WIDE), slice(None))

        pltpu.make_async_copy(obuf, o_hbm, out_sem).wait()

    out = pl.pallas_call(
        kernel,
        in_specs=[pl.BlockSpec(memory_space=pltpu.HBM)] * 3,
        out_specs=pl.BlockSpec(memory_space=pltpu.HBM),
        out_shape=jax.ShapeDtypeStruct(shape, x.dtype),
        scratch_shapes=[
            pltpu.VMEM(shape, x.dtype),
            pltpu.VMEM(shape, x.dtype),
            pltpu.VMEM((C,), g.dtype),
            pltpu.VMEM((C,), b.dtype),
            pltpu.SMEM((smem_rows, C), x.dtype),
            pltpu.SemaphoreType.DMA((_SETS,)),
            pltpu.SemaphoreType.DMA(()),
            pltpu.SemaphoreType.DMA(()),
            pltpu.SemaphoreType.DMA((2,)),
            pltpu.SemaphoreType.DMA((2,)),
            pltpu.SemaphoreType.DMA((P,)),
            pltpu.SemaphoreType.DMA(()),
        ],
        compiler_params=pltpu.CompilerParams(
            vmem_limit_bytes=64 * 2**20, disable_semaphore_checks=True),
    )(x.transpose(0, 2, 3, 1).reshape(shape), g, b)
    return out.reshape(B, H, W, C).transpose(0, 3, 1, 2)
```

```python
import jax
import jax.numpy as jnp
from jax import lax
import jax.experimental.pallas as pl
import jax.experimental.pallas.tpu as pltpu

_GROUPS = 32
_EPS = 1e-5

_SETS = 4
_EARLY_SETS = 2
_ROWS = 8
_DMA_ROWS = 24
_TAIL_ROWS = 48
_WIDE = 6
_SIDE_ROWS = 128
_SIDE_TWICE = 8
_SIDE_SPLIT = (0, 4, 5, _WIDE)


def _start_rows(copy, lo, hi):
    whole = (hi - lo) // _DMA_ROWS

    @pl.loop(0, whole)
    def _(j):
        copy(pl.multiple_of(lo + j * _DMA_ROWS, _ROWS), _DMA_ROWS).start()

    rest = lo + whole * _DMA_ROWS
    if rest < hi:
        copy(rest, hi - rest).start()


def _normalise(src, dst, member, gamma, beta):
    rows, C = src.shape
    count = rows * (C // _GROUPS)
    steps = [pl.ds(row, _ROWS) for row in range(0, rows, _ROWS)]

    def group_mean(partial):
        cols = jnp.sum(partial, axis=0, keepdims=True)
        return jnp.sum(jnp.where(member, cols, 0.0), axis=1, keepdims=True) / count

    def per_channel(v):
        return jnp.sum(jnp.where(member, v, 0.0), axis=0, keepdims=True)

    total = jnp.zeros((_ROWS, C), jnp.float32)
    for step in steps:
        total += src[step, :].astype(jnp.float32)
    mean = jnp.broadcast_to(per_channel(group_mean(total)), (_ROWS, C))

    squares = jnp.zeros((_ROWS, C), jnp.float32)
    for step in steps:
        d = src[step, :].astype(jnp.float32) - mean
        squares += d * d
    rstd = per_channel(lax.rsqrt(group_mean(squares) + _EPS))

    scale = jnp.broadcast_to(rstd * gamma, (_ROWS, C))
    shift = jnp.broadcast_to(beta, (_ROWS, C))
    for step in steps:
        d = src[step, :].astype(jnp.float32) - mean
        dst[step, :] = (d * scale + shift).astype(dst.dtype)


def _kernel(x_hbm, g_hbm, b_hbm, o_hbm, xbuf, obuf, gbuf, bbuf, side, out_sem):
    P, _, HW, C = x_hbm.shape
    last = _SETS - 1
    wide = pl.ds(0, _WIDE)
    narrow = pl.ds(_WIDE, P - _WIDE)
    side_start = HW - _SIDE_ROWS - 2 * _SIDE_TWICE
    kept_start = side_start + _SIDE_TWICE
    tail_start = side_start - _TAIL_ROWS
    pieces = list(zip(_SIDE_SPLIT[:-1], _SIDE_SPLIT[1:]))

    def start_write(samples, sets):
        def write(row, n):
            idx = (samples, sets, pl.ds(row, n))
            return pltpu.make_async_copy(obuf.at[idx], o_hbm.at[idx], out_sem)

        _start_rows(write, 0, HW)

    def read_and_normalise(set_sem, tail_sem, narrow_sem, param_sem, side_sem, drain_sem):
        def read(k, row, n, sem):
            idx = (slice(None), k, pl.ds(row, n))
            return pltpu.make_async_copy(x_hbm.at[idx], xbuf.at[idx], sem)

        def drain(n):
            samples = pl.ds(pieces[n][0], pieces[n][1] - pieces[n][0])
            return pltpu.make_async_copy(
                side.at[samples],
                xbuf.at[samples, last, pl.ds(kept_start, HW - kept_start)],
                drain_sem.at[n])

        twice = side.at[:, pl.ds(_SIDE_ROWS, _SIDE_TWICE)]
        early = (wide, last, pl.ds(side_start, _SIDE_TWICE))
        fill_early = pltpu.make_async_copy(x_hbm.at[early], twice, side_sem.at[0])
        drain_early = pltpu.make_async_copy(twice, xbuf.at[early], side_sem.at[1])
        fill_once = pltpu.make_async_copy(
            x_hbm.at[wide, last, pl.ds(kept_start, _SIDE_ROWS)],
            side.at[:, pl.ds(0, _SIDE_ROWS)], side_sem.at[2])
        fill_late = pltpu.make_async_copy(
            x_hbm.at[wide, last, pl.ds(HW - _SIDE_TWICE, _SIDE_TWICE)], twice, side_sem.at[3])
        direct = (narrow, last, pl.ds(side_start, HW - side_start))
        read_narrow = pltpu.make_async_copy(x_hbm.at[direct], xbuf.at[direct], narrow_sem)
        read_g = pltpu.make_async_copy(g_hbm, gbuf, param_sem.at[0])
        read_b = pltpu.make_async_copy(b_hbm, bbuf, param_sem.at[1])

        read(0, 0, _DMA_ROWS, set_sem.at[0]).start()
        fill_early.start()
        fill_once.start()
        for k in range(_SETS):
            _start_rows(lambda row, n: read(k, row, n, set_sem.at[k]),
                        _DMA_ROWS if k == 0 else 0, tail_start if k == last else HW)
            if k == 0:
                read_g.start()
                read_b.start()
                fill_early.wait()
                drain_early.start()
            if k == last - 1:
                read_narrow.start()
                drain_early.wait()
                fill_late.start()
        _start_rows(lambda row, n: read(last, row, n, tail_sem), tail_start, side_start)

        read_g.wait()
        read_b.wait()
        gamma = gbuf[...].astype(jnp.float32).reshape(1, C)
        beta = bbuf[...].astype(jnp.float32).reshape(1, C)
        first = lax.broadcasted_iota(jnp.int32, (_GROUPS, C), 0) * (C // _GROUPS)
        channel = lax.broadcasted_iota(jnp.int32, (_GROUPS, C), 1)
        member = (channel >= first) & (channel < first + C // _GROUPS)

        @pl.loop(0, _SETS * P)
        def _(t):
            k = t // P
            i = (t + _WIDE) % P

            @pl.when((t % P == 0) & (k < last))
            def _():
                read(k, 0, HW, set_sem.at[k]).wait()

            @pl.when(t == _EARLY_SETS * P)
            def _():
                fill_once.wait()
                fill_late.wait()
                for n in range(len(pieces)):
                    drain(n).start()
                read_narrow.wait()
                read(last, 0, tail_start, set_sem.at[last]).wait()
                for done in range(_EARLY_SETS):
                    start_write(wide, pl.ds(done, 1))
                read(last, tail_start, _TAIL_ROWS, tail_sem).wait()

            for n, (lo, _) in enumerate(pieces):
                @pl.when((k == last) & (i == lo))
                def _():
                    drain(n).wait()

            _normalise(xbuf.at[i, k], obuf.at[i, k], member, gamma, beta)

            @pl.when((t % P == P - 1) & (k >= _EARLY_SETS))
            def _():
                start_write(wide, pl.ds(k, 1))

            @pl.when((k == last) & (i == P - 1))
            def _():
                start_write(narrow, slice(None))

    dma = pltpu.SemaphoreType.DMA
    pl.run_scoped(read_and_normalise, dma((_SETS,)), dma(()), dma(()), dma((2,)),
                  dma((4,)), dma((len(pieces),)))
    pltpu.make_async_copy(obuf, o_hbm, out_sem).wait()


@jax.jit
def pallas_standalone__groupnorm__sampling_kernel(
    x: jax.Array,
    g: jax.Array,
    b: jax.Array,
):
    B, C, H, W = x.shape
    shape = (B // _SETS, _SETS, H * W, C)
    out = pl.pallas_call(
        _kernel,
        in_specs=[pl.BlockSpec(memory_space=pltpu.HBM)] * 3,
        out_specs=pl.BlockSpec(memory_space=pltpu.HBM),
        out_shape=jax.ShapeDtypeStruct(shape, x.dtype),
        scratch_shapes=[
            pltpu.VMEM(shape, x.dtype),
            pltpu.VMEM(shape, x.dtype),
            pltpu.VMEM((C,), g.dtype),
            pltpu.VMEM((C,), b.dtype),
            pltpu.SMEM((_WIDE, _SIDE_ROWS + _SIDE_TWICE, C), x.dtype),
            pltpu.SemaphoreType.DMA(()),
        ],
        compiler_params=pltpu.CompilerParams(vmem_limit_bytes=64 * 2**20),
    )(x.transpose(0, 2, 3, 1).reshape(shape), g, b)
    return out.reshape(B, H, W, C).transpose(0, 3, 1, 2)
```
